```python
import os as _os
_os.environ.setdefault("JAX_PLATFORMS", "cpu")
import jax
import jax.numpy as jnp

def _softmax(x, axis=-1):
    return jax.nn.softmax(x, axis=axis)
def _gelu(x):
    return jax.nn.gelu(x, approximate=True)
def _silu(x):
    return jax.nn.silu(x)
def _sigmoid(x):
    return jax.nn.sigmoid(x)
def _layernorm(x, axis=-1, eps=1e-5):
    m = jnp.mean(x, axis=axis, keepdims=True)
    v = jnp.var(x, axis=axis, keepdims=True)
    return (x - m) / jnp.sqrt(v + eps)
def _scatter_add(tgt, idx, src, axis=0):
    return tgt.at[idx].add(src)
def _segment_sum(src, seg, n):
    return jax.ops.segment_sum(src, seg, n)
class _Rng:
    def __init__(self, key):
        self._k = key
    def _next(self):
        self._k, sub = jax.random.split(self._k)
        return sub
    def normal(self, shape):
        return jax.random.normal(self._next(), shape, dtype=jnp.bfloat16)
    def randint(self, lo, hi, shape):
        return jax.random.randint(self._next(), shape, lo, hi, dtype=jnp.int32)
    def uniform(self, shape, lo=0.0, hi=1.0):
        return jax.random.uniform(self._next(), shape, jnp.bfloat16, lo, hi)
    def permutation(self, n):
        return jax.random.permutation(self._next(), n)


kernel_name = 'sequential_preLN__mha_block__mixer_token_mlp__prompt'

def setup_inputs():
    _rng = _Rng(jax.random.key(int.from_bytes(__import__("os").urandom(4), "little")))
    _w = (lambda a: (lambda t: t.astype(jnp.bfloat16) if jnp.issubdtype(t.dtype, jnp.floating) else t)(jnp.asarray(a)))
    def _A_setup():
        B, S, D, H = 1, 2048, 448, 16
        return {
            "x": _w((lambda *s: _rng.normal(s) * 0.05)(B, S, D)),
            "wqkv": _w((lambda *s: _rng.normal(s) * 0.05)(D, 3 * D)),
            "wo": _w((lambda *s: _rng.normal(s) * 0.05)(D, D)),
        }
    _A_in = _A_setup()

    def _B_setup():
        B, S, D, F = 1, 2048, 448, 1792
        return {
            "x": _w((lambda *s: _rng.normal(s) * 0.05)(B, S, D)),
            "w1": _w((lambda *s: _rng.normal(s) * 0.2)(S, F) * (S ** -0.5)),
            "b1": _w((lambda *s: _rng.normal(s) * 0.2)(F) * 0.02),
            "w2": _w((lambda *s: _rng.normal(s) * 0.2)(F, S) * (F ** -0.5)),
            "b2": _w((lambda *s: _rng.normal(s) * 0.05)(S) * 0.02),
        }
    _B_in = _B_setup()

    return {
        "A_x": _A_in["x"],
        "A_wqkv": _A_in["wqkv"],
        "A_wo": _A_in["wo"],
        "B_x": _B_in["x"],
        "B_w1": _B_in["w1"],
        "B_b1": _B_in["b1"],
        "B_w2": _B_in["w2"],
        "B_b2": _B_in["b2"],
    }

def reference(A_x, A_wqkv, A_wo, B_x, B_w1, B_b1, B_w2, B_b2):
    def _A_ref(x, wqkv, wo):
        B, S, D = x.shape
        H = 16
        Dh = D // H
        qkv = (lambda x, *d: x.transpose(*d))((x @ wqkv).reshape(B, S, 3, H, Dh), 2, 0, 3, 1, 4)
        q, k, v = qkv[0], qkv[1], qkv[2]
        scores = jnp.einsum("bhqd,bhkd->bhqk", q, k) * (Dh ** -0.5)
        p = _softmax(scores, axis=-1)
        o = jnp.einsum("bhqk,bhkd->bhqd", p, v)
        return (lambda x, *d: x.transpose(*d))(o, 0, 2, 1, 3).reshape(B, S, D) @ wo

    def _B_ref(x, w1, b1, w2, b2):
        B, S, D = x.shape
        h = _layernorm(x, axis=-1)
        u = jnp.einsum("bsd,sf->bdf", h, w1) + b1
        u = _gelu(u)
        y = jnp.einsum("bdf,fs->bds", u, w2) + b2
        return (lambda x, *d: x.transpose(*d))(y, 0, 2, 1)

    x = A_x
    h = x + _A_ref(_layernorm(x, axis=-1), A_wqkv, A_wo)
    h2 = h + _B_ref(_layernorm(h, axis=-1), B_w1, B_b1, B_w2, B_b2)
    return h2
```

```python
import functools
import math

import jax
import jax.numpy as jnp
import jax.experimental.pallas as pl
import jax.experimental.pallas.tpu as pltpu

S = 2048
D = 448
H = 16
DH = 28
DP = 32
HP = H * DP
F = 1792
EPS = 1e-5

TQ = 512
TK = 128
SHIFT = 3
UNROLL = 2
RC = 512
FC = 256
SC = 256

NT_DIMS = (((1,), (1,)), ((), ()))
BF = jnp.bfloat16
F32 = jnp.float32


def _expand_matrix(ncols, off):
    i = jax.lax.broadcasted_iota(jnp.int32, (HP, ncols), 0)
    k = jax.lax.broadcasted_iota(jnp.int32, (HP, ncols), 1)
    hit = jnp.logical_and((i % DP) < DH, k == off + DH * (i // DP) + (i % DP))
    return jnp.where(hit, 1.0, 0.0).astype(BF)


def _layernorm(v, axis):
    m = jnp.mean(v, axis=axis, keepdims=True)
    c = v - m
    var = jnp.mean(c * c, axis=axis, keepdims=True)
    return c * jax.lax.rsqrt(var + EPS)


def _gelu(u):
    c = math.sqrt(2.0 / math.pi)
    return 0.5 * u * (1.0 + jnp.tanh(c * (u + 0.044715 * (u * u * u))))


def _kernel(x_hbm, wqkv_hbm, wo_hbm, w1_hbm, b1_ref, w2_hbm, b2_ref, out_hbm,
            x_v, wqkv_v, wo_v, w1_v, w2_v,
            wqvT, wkp, woT,
            k_s, qT_s, vT_s, s0, s1, m0, m1, oT_s,
            hT_s, lnT_s, g_s, out_v, sems, osems):
    NRC = S // RC
    cp_wqkv = pltpu.make_async_copy(wqkv_hbm, wqkv_v, sems.at[0])
    cp_wqkv.start()
    cp_x = [pltpu.make_async_copy(x_hbm.at[0, pl.ds(c * RC, RC), :], x_v.at[pl.ds(c * RC, RC), :], sems.at[1 + c])
            for c in range(NRC)]
    for cp in cp_x:
        cp.start()
    cp_wo = pltpu.make_async_copy(wo_hbm, wo_v, sems.at[1 + NRC])
    cp_w1 = pltpu.make_async_copy(w1_hbm, w1_v, sems.at[2 + NRC])
    cp_w2 = pltpu.make_async_copy(w2_hbm, w2_v, sems.at[3 + NRC])
    cp_wo.start()
    cp_w1.start()
    cp_w2.start()

    cp_wqkv.wait()
    e0 = _expand_matrix(512, 0)
    wqvT[0:HP, :] = jax.lax.dot_general(e0, wqkv_v[:, 0:512], NT_DIMS,
                                        preferred_element_type=F32).astype(BF)
    ev = _expand_matrix(D, 0)
    wqvT[HP:2 * HP, :] = jax.lax.dot_general(ev, wqkv_v[:, 2 * D:3 * D], NT_DIMS,
                                             preferred_element_type=F32).astype(BF)
    ek = _expand_matrix(512, 64)
    wkp[...] = jax.lax.dot_general(wqkv_v[:, 384:896], ek, NT_DIMS,
                                   preferred_element_type=F32).astype(BF)

    qscale = (DH ** -0.5) * math.log2(math.e)
    row = jax.lax.broadcasted_iota(jnp.int32, (HP, RC), 0)
    ones_row = (row % DP) == DH
    for c in range(NRC):
        cp_x[c].wait()
        rows = slice(c * RC, (c + 1) * RC)
        xb = x_v[rows, :]
        hT_s[:, rows] = xb.T.astype(F32)
        xn = _layernorm(xb.astype(F32), -1).astype(BF)
        kc = jnp.dot(xn, wkp[...], preferred_element_type=F32).astype(BF)
        for h in range(H):
            k_s[h, rows, :] = kc[:, h * DP:(h + 1) * DP]
        qv = jax.lax.dot_general(wqvT[...], xn, NT_DIMS, preferred_element_type=F32)
        qT_s[:, rows] = (qv[0:HP] * qscale).astype(BF)
        vT_s[:, rows] = jnp.where(ones_row, 1.0, qv[HP:2 * HP]).astype(BF)

    cp_wo.wait()
    wo_pad = jnp.dot(ev, wo_v[...], preferred_element_type=F32).astype(BF)
    woT[...] = wo_pad.T

    NQ = S // TQ
    NTILE = H * NQ
    NC = S // TK
    sbuf = (s0, s1)
    mbuf = (m0, m1)

    def run(nsteps, tbase, acc, a_lim, b_lo, b_lim):
        q = ha = m8 = mb = None
        for n in range(nsteps):
            if n < a_lim:
                rt, c = divmod(n, NC)
                if c == 0:
                    t = tbase + rt
                    ha = t // NQ
                    qoff = pl.multiple_of((t % NQ) * TQ, TQ)
                    q = qT_s[pl.ds(pl.multiple_of(ha * DP, DP), DP), pl.ds(qoff, TQ)]
                    m8 = None
                s = jnp.dot(k_s[ha, c * TK:(c + 1) * TK, :], q, preferred_element_type=F32)
                sbuf[rt % 2][c * TK:(c + 1) * TK, :] = s
                mm = jnp.max(s.reshape(TK // 8, 8, TQ), axis=0)
                m8 = mm if m8 is None else jnp.maximum(m8, mm)
                if c == NC - 1:
                    mbuf[rt % 2][...] = jnp.max(m8, axis=0, keepdims=True)
            b = n - NC - SHIFT
            if b_lo <= b < b_lim:
                rt, c = divmod(b, NC)
                t = tbase + rt
                hoff = pl.multiple_of((t // NQ) * DP, DP)
                if c == 0 or mb is None:
                    mb = mbuf[rt % 2][...]
                p = jnp.exp2(sbuf[rt % 2][c * TK:(c + 1) * TK, :] - mb).astype(BF)
                o = jnp.dot(vT_s[pl.ds(hoff, DP), c * TK:(c + 1) * TK], p, preferred_element_type=F32)
                acc = o if c == 0 else acc + o
                if c == NC - 1:
                    qoff = pl.multiple_of((t % NQ) * TQ, TQ)
                    oT_s[pl.ds(hoff, DP), pl.ds(qoff, TQ)] = (acc / acc[DH:DH + 1, :]).astype(BF)
                    mb = None
        return acc

    big = 1 << 30
    acc0 = run(2 * NC, 0, None, big, 0, big)

    def attn_body(i, acc):
        return run(UNROLL * NC, 2 + i * UNROLL, acc, big, -big, big)

    nit = (NTILE - 2) // UNROLL
    acc1 = jax.lax.fori_loop(0, nit, attn_body, acc0)
    rem = (NTILE - 2) - nit * UNROLL
    run(rem * NC + NC + SHIFT, 2 + nit * UNROLL, acc1, rem * NC, -big, rem * NC)

    for c in range(S // RC):
        cols = slice(c * RC, (c + 1) * RC)
        hT = hT_s[:, cols] + jnp.dot(woT[...], oT_s[:, cols], preferred_element_type=F32)
        hT_s[:, cols] = hT
        lnT_s[:, cols] = _layernorm(hT, 0).astype(BF)

    cp_w1.wait()
    b1 = b1_ref[...].astype(F32).reshape(1, F)
    for c in range(F // FC):
        cols = slice(c * FC, (c + 1) * FC)
        u = jnp.dot(lnT_s[...], w1_v[:, cols], preferred_element_type=F32) + b1[:, cols]
        g_s[:, cols] = _gelu(u).astype(BF)

    cp_w2.wait()
    b2 = b2_ref[...].astype(F32).reshape(1, S)
    ocp = []
    for c in range(S // SC):
        cols = slice(c * SC, (c + 1) * SC)
        y = jnp.dot(g_s[...], w2_v[:, cols], preferred_element_type=F32) + b2[:, cols]
        res = (hT_s[:, cols] + y).astype(BF)
        out_v[cols, :] = res.T
        cp = pltpu.make_async_copy(out_v.at[pl.ds(c * SC, SC), :], out_hbm.at[0, pl.ds(c * SC, SC), :], osems.at[c])
        cp.start()
        ocp.append(cp)
    for cp in ocp:
        cp.wait()


@jax.jit
def pallas_sequential_preLN__mha_block__mixer_token_mlp__prompt_kernel(
    A_x: jax.Array,
    A_wqkv: jax.Array,
    A_wo: jax.Array,
    B_x: jax.Array,
    B_w1: jax.Array,
    B_b1: jax.Array,
    B_w2: jax.Array,
    B_b2: jax.Array,
):
    del B_x
    any_spec = pl.BlockSpec(memory_space=pl.ANY)
    vmem_spec = pl.BlockSpec(memory_space=pltpu.VMEM)
    scratch = [
        pltpu.VMEM((S, D), BF),
        pltpu.VMEM((D, 3 * D), BF),
        pltpu.VMEM((D, D), BF),
        pltpu.VMEM((S, F), BF),
        pltpu.VMEM((F, S), BF),
        pltpu.VMEM((2 * HP, D), BF),
        pltpu.VMEM((D, HP), BF),
        pltpu.VMEM((D, HP), BF),
        pltpu.VMEM((H, S, DP), BF),
        pltpu.VMEM((HP, S), BF),
        pltpu.VMEM((HP, S), BF),
        pltpu.VMEM((S, TQ), F32),
        pltpu.VMEM((S, TQ), F32),
        pltpu.VMEM((1, TQ), F32),
        pltpu.VMEM((1, TQ), F32),
        pltpu.VMEM((HP, S), BF),
        pltpu.VMEM((D, S), F32),
        pltpu.VMEM((D, S), BF),
        pltpu.VMEM((D, F), BF),
        pltpu.VMEM((S, D), BF),
        pltpu.SemaphoreType.DMA((4 + S // RC,)),
        pltpu.SemaphoreType.DMA((S // SC,)),
    ]
    return pl.pallas_call(
        _kernel,
        out_shape=jax.ShapeDtypeStruct((1, S, D), BF),
        in_specs=[any_spec, any_spec, any_spec, any_spec, vmem_spec, any_spec, vmem_spec],
        out_specs=any_spec,
        scratch_shapes=scratch,
        compiler_params=pltpu.CompilerParams(vmem_limit_bytes=110 * 1024 * 1024),
    )(A_x, A_wqkv, A_wo, B_w1, B_b1, B_w2, B_b2)
```

```python
import functools
import math

import jax
import jax.numpy as jnp
import jax.experimental.pallas as pl
import jax.experimental.pallas.tpu as pltpu

S = 2048
D = 448
H = 16
DH = 28
DP = 32
HP = H * DP
F = 1792
EPS = 1e-5

TQ = 512
TK = 128
SHIFT = 3
UNROLL = 2
RC = 512
FC = 256
SC = 256

NT_DIMS = (((1,), (1,)), ((), ()))
BF = jnp.bfloat16
F32 = jnp.float32


def _expand_matrix(ncols, off):
    i = jax.lax.broadcasted_iota(jnp.int32, (HP, ncols), 0)
    k = jax.lax.broadcasted_iota(jnp.int32, (HP, ncols), 1)
    hit = jnp.logical_and((i % DP) < DH, k == off + DH * (i // DP) + (i % DP))
    return jnp.where(hit, 1.0, 0.0).astype(BF)


def _layernorm(v, axis):
    m = jnp.mean(v, axis=axis, keepdims=True)
    c = v - m
    var = jnp.mean(c * c, axis=axis, keepdims=True)
    return c * jax.lax.rsqrt(var + EPS)


def _gelu(u):
    c = math.sqrt(2.0 / math.pi)
    return 0.5 * u * (1.0 + jnp.tanh(c * (u + 0.044715 * (u * u * u))))


def _kernel(x_hbm, wqkv_hbm, wo_hbm, w1_hbm, b1_ref, w2_hbm, b2_ref, out_hbm,
            x_v, wqkv_v, wo_v, w1_v, w2_v,
            wT, woT,
            k_s, qT_s, vT_s, s0, s1, m0, m1, oT_s,
            hT_s, lnT_s, g_s, out_v, sems, osems):
    NRC = S // RC
    cp_wqkv = pltpu.make_async_copy(wqkv_hbm, wqkv_v, sems.at[0])
    cp_wqkv.start()
    cp_x = [pltpu.make_async_copy(x_hbm.at[0, :, pl.ds(c * RC, RC)], x_v.at[:, pl.ds(c * RC, RC)], sems.at[1 + c])
            for c in range(NRC)]
    for cp in cp_x:
        cp.start()
    cp_wo = pltpu.make_async_copy(wo_hbm, wo_v, sems.at[1 + NRC])
    cp_w1 = pltpu.make_async_copy(w1_hbm, w1_v, sems.at[2 + NRC])
    cp_w2 = pltpu.make_async_copy(w2_hbm, w2_v, sems.at[3 + NRC])
    cp_wo.start()
    cp_w1.start()
    cp_w2.start()

    cp_wqkv.wait()
    e0 = _expand_matrix(512, 0)
    wT[0:HP, :] = jax.lax.dot_general(e0, wqkv_v[:, 0:512], NT_DIMS,
                                      preferred_element_type=F32).astype(BF)
    ek = _expand_matrix(512, 64)
    wT[HP:2 * HP, :] = jax.lax.dot_general(ek, wqkv_v[:, 384:896], NT_DIMS,
                                           preferred_element_type=F32).astype(BF)
    ev = _expand_matrix(D, 0)
    wT[2 * HP:3 * HP, :] = jax.lax.dot_general(ev, wqkv_v[:, 2 * D:3 * D], NT_DIMS,
                                               preferred_element_type=F32).astype(BF)

    qscale = (DH ** -0.5) * math.log2(math.e)
    row = jax.lax.broadcasted_iota(jnp.int32, (HP, RC), 0)
    ones_row = (row % DP) == DH
    for c in range(NRC):
        cp_x[c].wait()
        cols = slice(c * RC, (c + 1) * RC)
        xn = _layernorm(x_v[:, cols].astype(F32), 0).astype(BF)
        qkv = jnp.dot(wT[...], xn, preferred_element_type=F32)
        qT_s[:, cols] = (qkv[0:HP] * qscale).astype(BF)
        kt = qkv[HP:2 * HP].astype(BF)
        for h in range(H):
            k_s[h, cols, :] = kt[h * DP:(h + 1) * DP, :].T
        vT_s[:, cols] = jnp.where(ones_row, 1.0, qkv[2 * HP:3 * HP]).astype(BF)

    cp_wo.wait()
    wo_pad = jnp.dot(ev, wo_v[...], preferred_element_type=F32).astype(BF)
    woT[...] = wo_pad.T

    NQ = S // TQ
    NTILE = H * NQ
    NC = S // TK
    sbuf = (s0, s1)
    mbuf = (m0, m1)

    def run(nsteps, tbase, acc, a_lim, b_lo, b_lim):
        q = ha = m8 = mb = None
        for n in range(nsteps):
            if n < a_lim:
                rt, c = divmod(n, NC)
                if c == 0:
                    t = tbase + rt
                    ha = t // NQ
                    qoff = pl.multiple_of((t % NQ) * TQ, TQ)
                    q = qT_s[pl.ds(pl.multiple_of(ha * DP, DP), DP), pl.ds(qoff, TQ)]
                    m8 = None
                s = jnp.dot(k_s[ha, c * TK:(c + 1) * TK, :], q, preferred_element_type=F32)
                sbuf[rt % 2][c * TK:(c + 1) * TK, :] = s
                mm = jnp.max(s.reshape(TK // 8, 8, TQ), axis=0)
                m8 = mm if m8 is None else jnp.maximum(m8, mm)
                if c == NC - 1:
                    mbuf[rt % 2][...] = jnp.max(m8, axis=0, keepdims=True)
            b = n - NC - SHIFT
            if b_lo <= b < b_lim:
                rt, c = divmod(b, NC)
                t = tbase + rt
                hoff = pl.multiple_of((t // NQ) * DP, DP)
                if c == 0 or mb is None:
                    mb = mbuf[rt % 2][...]
                p = jnp.exp2(sbuf[rt % 2][c * TK:(c + 1) * TK, :] - mb).astype(BF)
                o = jnp.dot(vT_s[pl.ds(hoff, DP), c * TK:(c + 1) * TK], p, preferred_element_type=F32)
                acc = o if c == 0 else acc + o
                if c == NC - 1:
                    qoff = pl.multiple_of((t % NQ) * TQ, TQ)
                    oT_s[pl.ds(hoff, DP), pl.ds(qoff, TQ)] = (acc / acc[DH:DH + 1, :]).astype(BF)
                    mb = None
        return acc

    big = 1 << 30
    acc0 = run(2 * NC, 0, None, big, 0, big)

    def attn_body(i, acc):
        return run(UNROLL * NC, 2 + i * UNROLL, acc, big, -big, big)

    nit = (NTILE - 2) // UNROLL
    acc1 = jax.lax.fori_loop(0, nit, attn_body, acc0)
    rem = (NTILE - 2) - nit * UNROLL
    run(rem * NC + NC + SHIFT, 2 + nit * UNROLL, acc1, rem * NC, -big, rem * NC)

    for c in range(S // RC):
        cols = slice(c * RC, (c + 1) * RC)
        hT = x_v[:, cols].astype(F32) + jnp.dot(woT[...], oT_s[:, cols], preferred_element_type=F32)
        hT_s[:, cols] = hT
        lnT_s[:, cols] = _layernorm(hT, 0).astype(BF)

    cp_w1.wait()
    b1 = b1_ref[...].astype(F32).reshape(1, F)
    for c in range(F // FC):
        cols = slice(c * FC, (c + 1) * FC)
        u = jnp.dot(lnT_s[...], w1_v[:, cols], preferred_element_type=F32) + b1[:, cols]
        g_s[:, cols] = _gelu(u).astype(BF)

    cp_w2.wait()
    b2 = b2_ref[...].astype(F32).reshape(1, S)
    ocp = []
    for c in range(S // SC):
        cols = slice(c * SC, (c + 1) * SC)
        y = jnp.dot(g_s[...], w2_v[:, cols], preferred_element_type=F32) + b2[:, cols]
        out_v[:, cols] = (hT_s[:, cols] + y).astype(BF)
        cp = pltpu.make_async_copy(out_v.at[:, pl.ds(c * SC, SC)], out_hbm.at[0, :, pl.ds(c * SC, SC)], osems.at[c])
        cp.start()
        ocp.append(cp)
    for cp in ocp:
        cp.wait()


@jax.jit
def pallas_sequential_preLN__mha_block__mixer_token_mlp__prompt_kernel(
    A_x: jax.Array,
    A_wqkv: jax.Array,
    A_wo: jax.Array,
    B_x: jax.Array,
    B_w1: jax.Array,
    B_b1: jax.Array,
    B_w2: jax.Array,
    B_b2: jax.Array,
):
    del B_x
    hbm_spec = pl.BlockSpec(memory_space=pltpu.MemorySpace.HBM)
    vmem_spec = pl.BlockSpec(memory_space=pltpu.VMEM)
    scratch = [
        pltpu.VMEM((D, S), BF),
        pltpu.VMEM((D, 3 * D), BF),
        pltpu.VMEM((D, D), BF),
        pltpu.VMEM((S, F), BF),
        pltpu.VMEM((F, S), BF),
        pltpu.VMEM((3 * HP, D), BF),
        pltpu.VMEM((D, HP), BF),
        pltpu.VMEM((H, S, DP), BF),
        pltpu.VMEM((HP, S), BF),
        pltpu.VMEM((HP, S), BF),
        pltpu.VMEM((S, TQ), F32),
        pltpu.VMEM((S, TQ), F32),
        pltpu.VMEM((1, TQ), F32),
        pltpu.VMEM((1, TQ), F32),
        pltpu.VMEM((HP, S), BF),
        pltpu.VMEM((D, S), F32),
        pltpu.VMEM((D, S), BF),
        pltpu.VMEM((D, F), BF),
        pltpu.VMEM((D, S), BF),
        pltpu.SemaphoreType.DMA((4 + S // RC,)),
        pltpu.SemaphoreType.DMA((S // SC,)),
    ]
    xT = jnp.swapaxes(A_x, 1, 2)
    outT = pl.pallas_call(
        _kernel,
        out_shape=jax.ShapeDtypeStruct((1, D, S), BF),
        in_specs=[hbm_spec, hbm_spec, hbm_spec, hbm_spec, vmem_spec, hbm_spec, vmem_spec],
        out_specs=hbm_spec,
        scratch_shapes=scratch,
        compiler_params=pltpu.CompilerParams(vmem_limit_bytes=110 * 1024 * 1024),
    )(xT, A_wqkv, A_wo, B_w1, B_b1, B_w2, B_b2)
    return jnp.swapaxes(outT, 1, 2)
```

```python
import functools
import math

import jax
import jax.numpy as jnp
import jax.experimental.pallas as pl
import jax.experimental.pallas.tpu as pltpu

S = 2048
D = 448
H = 16
DH = 28
DP = 32
HP = H * DP
F = 1792
EPS = 1e-5

TQ = 512
TK = 128
SHIFT = 3
UNROLL = 2
RC = 512
FC = 256
SC = 256

NT_DIMS = (((1,), (1,)), ((), ()))
BF = jnp.bfloat16
F32 = jnp.float32


def _expand_matrix(ncols, off):
    i = jax.lax.broadcasted_iota(jnp.int32, (HP, ncols), 0)
    k = jax.lax.broadcasted_iota(jnp.int32, (HP, ncols), 1)
    hit = jnp.logical_and((i % DP) < DH, k == off + DH * (i // DP) + (i % DP))
    return jnp.where(hit, 1.0, 0.0).astype(BF)


def _layernorm(v, axis):
    m = jnp.mean(v, axis=axis, keepdims=True)
    c = v - m
    var = jnp.mean(c * c, axis=axis, keepdims=True)
    return c * jax.lax.rsqrt(var + EPS)


def _gelu(u):
    c = math.sqrt(2.0 / math.pi)
    return 0.5 * u * (1.0 + jnp.tanh(c * (u + 0.044715 * (u * u * u))))


def _kernel(x_hbm, wqkv_hbm, wo_hbm, w1_hbm, b1_ref, w2_hbm, b2_ref, out_hbm,
            x_v, wqkv_v, wo_v, w1_v, w2_v,
            wT, wop, woT,
            k_s, qT_s, vT_s, s0, s1, m0, m1, oT_s,
            hT_s, lnT_s, g_s, out_v, sems, osems):
    NRC = S // RC
    cp_x = [pltpu.make_async_copy(x_hbm.at[0, :, pl.ds(c * RC, RC)], x_v.at[:, pl.ds(c * RC, RC)], sems.at[1 + c])
            for c in range(NRC)]
    cp_wqkv = pltpu.make_async_copy(wqkv_hbm, wqkv_v, sems.at[0])
    cp_wo = pltpu.make_async_copy(wo_hbm, wo_v, sems.at[1 + NRC])
    cp_w1 = pltpu.make_async_copy(w1_hbm, w1_v, sems.at[2 + NRC])
    cp_w2 = pltpu.make_async_copy(w2_hbm, w2_v, sems.at[3 + NRC])
    cp_wqkv.start()
    cp_x[0].start()
    for cp in cp_x[1:]:
        cp.start()
    cp_wo.start()

    qscale = (DH ** -0.5) * math.log2(math.e)

    def project(c):
        cols = slice(c * RC, (c + 1) * RC)
        xn = _layernorm(x_v[:, cols].astype(F32), 0).astype(BF)
        qkv = jnp.dot(wT[...], xn, preferred_element_type=F32)
        for h in range(H):
            qT_s[h * DP:h * DP + DH, cols] = (qkv[h * DH:(h + 1) * DH] * qscale).astype(BF)
            k_s[h, cols, :] = qkv[D + h * DH:D + (h + 1) * DH].astype(BF).T
            vT_s[h * DP:h * DP + DH, cols] = qkv[2 * D + h * DH:2 * D + (h + 1) * DH].astype(BF)

    cp_wqkv.wait()
    cp_x[0].wait()
    for j in range(3 * D // 128):
        wT[j * 128:(j + 1) * 128, :] = wqkv_v[:, j * 128:(j + 1) * 128].T
    wT[(3 * D // 128) * 128:3 * D, :] = wqkv_v[:, (3 * D // 128) * 128:3 * D].T
    prow = jax.lax.broadcasted_iota(jnp.int32, (DP - DH, S), 0)
    pad_rows = jnp.where(prow == 0, 1.0, 0.0).astype(BF)
    for h in range(H):
        vT_s[h * DP + DH:(h + 1) * DP, :] = pad_rows
    project(0)

    for cp in cp_x[1:]:
        cp.wait()
    cp_wo.wait()
    cp_w1.start()
    cp_w2.start()
    for h in range(H):
        wop[h * DP:h * DP + DH, :] = wo_v[h * DH:(h + 1) * DH, :]
        wop[h * DP + DH:(h + 1) * DP, :] = jnp.zeros((DP - DH, D), BF)
    woT[...] = wop[...].T
    for c in range(1, NRC):
        project(c)

    NQ = S // TQ
    NTILE = H * NQ
    NC = S // TK
    sbuf = (s0, s1)
    mbuf = (m0, m1)

    def run(nsteps, tbase, acc, a_lim, b_lo, b_lim):
        q = ha = m8 = mb = None
        for n in range(nsteps):
            if n < a_lim:
                rt, c = divmod(n, NC)
                if c == 0:
                    t = tbase + rt
                    ha = t // NQ
                    qoff = pl.multiple_of((t % NQ) * TQ, TQ)
                    q = qT_s[pl.ds(pl.multiple_of(ha * DP, DP), DH), pl.ds(qoff, TQ)]
                    m8 = None
                s = jnp.dot(k_s[ha, c * TK:(c + 1) * TK, :], q, preferred_element_type=F32)
                sbuf[rt % 2][c * TK:(c + 1) * TK, :] = s
                mm = jnp.max(s.reshape(TK // 8, 8, TQ), axis=0)
                m8 = mm if m8 is None else jnp.maximum(m8, mm)
                if c == NC - 1:
                    mbuf[rt % 2][...] = jnp.max(m8, axis=0, keepdims=True)
            b = n - NC - SHIFT
            if b_lo <= b < b_lim:
                rt, c = divmod(b, NC)
                t = tbase + rt
                hoff = pl.multiple_of((t // NQ) * DP, DP)
                if c == 0 or mb is None:
                    mb = mbuf[rt % 2][...]
                p = jnp.exp2(sbuf[rt % 2][c * TK:(c + 1) * TK, :] - mb).astype(BF)
                o = jnp.dot(vT_s[pl.ds(hoff, DP), c * TK:(c + 1) * TK], p, preferred_element_type=F32)
                acc = o if c == 0 else acc + o
                if c == NC - 1:
                    qoff = pl.multiple_of((t % NQ) * TQ, TQ)
                    oT_s[pl.ds(hoff, DP), pl.ds(qoff, TQ)] = (acc / acc[DH:DH + 1, :]).astype(BF)
                    mb = None
        return acc

    big = 1 << 30
    acc0 = run(2 * NC, 0, None, big, 0, big)

    def attn_body(i, acc):
        return run(UNROLL * NC, 2 + i * UNROLL, acc, big, -big, big)

    nit = (NTILE - 2) // UNROLL
    acc1 = jax.lax.fori_loop(0, nit, attn_body, acc0)
    rem = (NTILE - 2) - nit * UNROLL
    run(rem * NC + NC + SHIFT, 2 + nit * UNROLL, acc1, rem * NC, -big, rem * NC)

    for c in range(S // RC):
        cols = slice(c * RC, (c + 1) * RC)
        hT = x_v[:, cols].astype(F32) + jnp.dot(woT[...], oT_s[:, cols], preferred_element_type=F32)
        hT_s[:, cols] = hT
        lnT_s[:, cols] = _layernorm(hT, 0).astype(BF)

    cp_w1.wait()
    b1 = b1_ref[...].astype(F32).reshape(1, F)
    for c in range(F // FC):
        cols = slice(c * FC, (c + 1) * FC)
        u = jnp.dot(lnT_s[...], w1_v[:, cols], preferred_element_type=F32) + b1[:, cols]
        g_s[:, cols] = _gelu(u).astype(BF)

    cp_w2.wait()
    b2 = b2_ref[...].astype(F32).reshape(1, S)
    ocp = []
    for c in range(S // SC):
        cols = slice(c * SC, (c + 1) * SC)
        y = jnp.dot(g_s[...], w2_v[:, cols], preferred_element_type=F32) + b2[:, cols]
        out_v[:, cols] = (hT_s[:, cols] + y).astype(BF)
        cp = pltpu.make_async_copy(out_v.at[:, pl.ds(c * SC, SC)], out_hbm.at[0, :, pl.ds(c * SC, SC)], osems.at[c])
        cp.start()
        ocp.append(cp)
    for cp in ocp:
        cp.wait()


@jax.jit
def pallas_sequential_preLN__mha_block__mixer_token_mlp__prompt_kernel(
    A_x: jax.Array,
    A_wqkv: jax.Array,
    A_wo: jax.Array,
    B_x: jax.Array,
    B_w1: jax.Array,
    B_b1: jax.Array,
    B_w2: jax.Array,
    B_b2: jax.Array,
):
    del B_x
    hbm_spec = pl.BlockSpec(memory_space=pltpu.MemorySpace.HBM)
    vmem_spec = pl.BlockSpec(memory_space=pltpu.VMEM)
    scratch = [
        pltpu.VMEM((D, S), BF),
        pltpu.VMEM((D, 3 * D), BF),
        pltpu.VMEM((D, D), BF),
        pltpu.VMEM((S, F), BF),
        pltpu.VMEM((F, S), BF),
        pltpu.VMEM((3 * D, D), BF),
        pltpu.VMEM((HP, D), BF),
        pltpu.VMEM((D, HP), BF),
        pltpu.VMEM((H, S, DH), BF),
        pltpu.VMEM((HP, S), BF),
        pltpu.VMEM((HP, S), BF),
        pltpu.VMEM((S, TQ), F32),
        pltpu.VMEM((S, TQ), F32),
        pltpu.VMEM((1, TQ), F32),
        pltpu.VMEM((1, TQ), F32),
        pltpu.VMEM((HP, S), BF),
        pltpu.VMEM((D, S), F32),
        pltpu.VMEM((D, S), BF),
        pltpu.VMEM((D, F), BF),
        pltpu.VMEM((D, S), BF),
        pltpu.SemaphoreType.DMA((4 + S // RC,)),
        pltpu.SemaphoreType.DMA((S // SC,)),
    ]
    xT = jnp.swapaxes(A_x, 1, 2)
    outT = pl.pallas_call(
        _kernel,
        out_shape=jax.ShapeDtypeStruct((1, D, S), BF),
        in_specs=[hbm_spec, hbm_spec, hbm_spec, hbm_spec, vmem_spec, hbm_spec, vmem_spec],
        out_specs=hbm_spec,
        scratch_shapes=scratch,
        compiler_params=pltpu.CompilerParams(vmem_limit_bytes=110 * 1024 * 1024),
    )(xT, A_wqkv, A_wo, B_w1, B_b1, B_w2, B_b2)
    return jnp.swapaxes(outT, 1, 2)
```

```python
import math

import jax
import jax.numpy as jnp
import jax.experimental.pallas as pl
import jax.experimental.pallas.tpu as pltpu

S = 2048
D = 448
H = 16
DH = 28
DP = 32
HP = H * DP
F = 1792
EPS = 1e-5

TQ = 256
TK = 256
SHIFT = 3
UNROLL = 18
RC = 512
FC = 256
SC = 256

BF = jnp.bfloat16
F32 = jnp.float32


def _layernorm(v, axis):
    m = jnp.mean(v, axis=axis, keepdims=True)
    c = v - m
    var = jnp.mean(c * c, axis=axis, keepdims=True)
    return c * jax.lax.rsqrt(var + EPS)


def _gelu(u):
    c = math.sqrt(2.0 / math.pi)
    return 0.5 * u * (1.0 + jnp.tanh(c * (u + 0.044715 * (u * u * u))))


def _kernel(x_hbm, wqkv_hbm, wo_hbm, w1_hbm, b1_ref, w2_hbm, b2_ref, out_hbm,
            x_v, wqkv_v, wo_v, w1_v, w2_v,
            wT, wop, woT, xn_s,
            k_s, qT_s, vT_s, s0, s1, m0, m1, oT_s,
            hT_s, lnT_s, g_s, out_v, sems, osems):
    NRC = S // RC
    cp_x = [pltpu.make_async_copy(x_hbm.at[0, :, pl.ds(c * RC, RC)], x_v.at[:, pl.ds(c * RC, RC)], sems.at[c])
            for c in range(NRC)]
    wsplit = (0, 512, 896, 3 * D)
    cp_w = [pltpu.make_async_copy(wqkv_hbm.at[:, pl.ds(wsplit[i], wsplit[i + 1] - wsplit[i])],
                                  wqkv_v.at[:, pl.ds(wsplit[i], wsplit[i + 1] - wsplit[i])], sems.at[NRC + i])
            for i in range(3)]
    cp_wo = pltpu.make_async_copy(wo_hbm, wo_v, sems.at[NRC + 3])
    cp_w1 = pltpu.make_async_copy(w1_hbm, w1_v, sems.at[NRC + 4])
    cp_w2 = pltpu.make_async_copy(w2_hbm, w2_v, sems.at[NRC + 5])
    for cp in [cp_x[0], cp_w[0], cp_x[1], cp_w[1], cp_w[2]] + cp_x[2:] + [cp_wo, cp_w1, cp_w2]:
        cp.start()

    qscale = (DH ** -0.5) * math.log2(math.e)

    def transpose_w(lo, hi):
        for j in range(lo, hi, 128):
            e = min(j + 128, hi)
            wT[j:e, :] = wqkv_v[:, j:e].T

    def ln1(c):
        return _layernorm(x_v[:, c * RC:(c + 1) * RC].astype(F32), 0).astype(BF)

    def project_q(c, xn, h0=0, h1=H):
        cols = slice(c * RC, (c + 1) * RC)
        q = jnp.dot(wT[h0 * DH:h1 * DH, :], xn, preferred_element_type=F32)
        for h in range(h0, h1):
            r = (h - h0) * DH
            qT_s[h * DP:h * DP + DH, cols] = (q[r:r + DH] * qscale).astype(BF)

    def project_kv(c, xn):
        cols = slice(c * RC, (c + 1) * RC)
        kv = jnp.dot(wT[D:3 * D, :], xn, preferred_element_type=F32)
        for h in range(H):
            k_s[h, cols, :] = kv[h * DH:(h + 1) * DH].astype(BF).T
            vT_s[h * DP:h * DP + DH, cols] = kv[D + h * DH:D + (h + 1) * DH].astype(BF)

    cp_x[0].wait()
    xn_s[0] = ln1(0)
    prow = jax.lax.broadcasted_iota(jnp.int32, (DP - DH, S), 0)
    pad_rows = jnp.where(prow == 0, 1.0, 0.0).astype(BF)
    for h in range(H):
        vT_s[h * DP + DH:(h + 1) * DP, :] = pad_rows

    cp_w[0].wait()
    transpose_w(0, 512)
    project_q(0, xn_s[0], 0, H // 2)

    cp_x[1].wait()
    project_q(0, xn_s[0], H // 2, H)
    xn_s[1] = ln1(1)
    project_q(1, xn_s[1], 0, H // 2)

    cp_w[1].wait()
    cp_w[2].wait()
    project_q(1, xn_s[1], H // 2, H)
    transpose_w(512, 3 * D)
    project_kv(0, xn_s[0])

    for cp in cp_x[2:]:
        cp.wait()
    cp_wo.wait()
    project_kv(1, xn_s[1])
    for c in range(2, NRC):
        xn = ln1(c)
        project_q(c, xn)
        project_kv(c, xn)
    for h in range(H):
        wop[h * DP:h * DP + DH, :] = wo_v[h * DH:(h + 1) * DH, :]
        wop[h * DP + DH:(h + 1) * DP, :] = jnp.zeros((DP - DH, D), BF)
    woT[...] = wop[...].T

    NQ = S // TQ
    NTILE = H * NQ
    NC = S // TK
    sbuf = (s0, s1)
    mbuf = (m0, m1)

    def run(nsteps, tbase, acc, a_lim, b_lo, b_lim):
        q = ha = m8 = mb = None
        for n in range(nsteps):
            if n < a_lim:
                rt, c = divmod(n, NC)
                if c == 0:
                    t = tbase + rt
                    ha = t // NQ
                    qoff = pl.multiple_of((t % NQ) * TQ, TQ)
                    q = qT_s[pl.ds(pl.multiple_of(ha * DP, DP), DH), pl.ds(qoff, TQ)]
                    m8 = None
                s = jnp.dot(k_s[ha, c * TK:(c + 1) * TK, :], q, preferred_element_type=F32)
                sbuf[rt % 2][c * TK:(c + 1) * TK, :] = s
                mm = jnp.max(s.reshape(TK // 8, 8, TQ), axis=0)
                m8 = mm if m8 is None else jnp.maximum(m8, mm)
                if c == NC - 1:
                    mbuf[rt % 2][...] = jnp.max(m8, axis=0, keepdims=True)
            b = n - NC - SHIFT
            if b_lo <= b < b_lim:
                rt, c = divmod(b, NC)
                t = tbase + rt
                hoff = pl.multiple_of((t // NQ) * DP, DP)
                if c == 0 or mb is None:
                    mb = mbuf[rt % 2][...]
                p = jnp.exp2(sbuf[rt % 2][c * TK:(c + 1) * TK, :] - mb).astype(BF)
                o = jnp.dot(vT_s[pl.ds(hoff, DP), c * TK:(c + 1) * TK], p, preferred_element_type=F32)
                acc = o if c == 0 else acc + o
                if c == NC - 1:
                    qoff = pl.multiple_of((t % NQ) * TQ, TQ)
                    oT_s[pl.ds(hoff, DP), pl.ds(qoff, TQ)] = (acc / acc[DH:DH + 1, :]).astype(BF)
                    mb = None
        return acc

    big = 1 << 30
    acc0 = run(2 * NC, 0, None, big, 0, big)

    def attn_body(i, acc):
        return run(UNROLL * NC, 2 + i * UNROLL, acc, big, -big, big)

    nit = (NTILE - 2) // UNROLL
    acc1 = jax.lax.fori_loop(0, nit, attn_body, acc0)
    cp_w1.wait()
    cp_w2.wait()
    rem = (NTILE - 2) - nit * UNROLL
    run(rem * NC + NC + SHIFT, 2 + nit * UNROLL, acc1, rem * NC, -big, rem * NC)

    b1 = b1_ref[...].astype(F32).reshape(1, F)
    for c in range(S // RC):
        cols = slice(c * RC, (c + 1) * RC)
        hT = x_v[:, cols].astype(F32) + jnp.dot(woT[...], oT_s[:, cols], preferred_element_type=F32)
        hT_s[:, cols] = hT
        lnT_s[:, cols] = _layernorm(hT, 0).astype(BF)

    for e in range(F // FC):
        cols = slice(e * FC, (e + 1) * FC)
        u = jnp.dot(lnT_s[...], w1_v[:, cols], preferred_element_type=F32) + b1[:, cols]
        g_s[:, cols] = _gelu(u).astype(BF)

    b2 = b2_ref[...].astype(F32).reshape(1, S)
    ocp = []
    for c in range(S // SC):
        cols = slice(c * SC, (c + 1) * SC)
        y = jnp.dot(g_s[...], w2_v[:, cols], preferred_element_type=F32) + b2[:, cols]
        out_v[:, cols] = (hT_s[:, cols] + y).astype(BF)
        cp = pltpu.make_async_copy(out_v.at[:, pl.ds(c * SC, SC)], out_hbm.at[0, :, pl.ds(c * SC, SC)], osems.at[c])
        cp.start()
        ocp.append(cp)
    for cp in ocp:
        cp.wait()


@jax.jit
def pallas_sequential_preLN__mha_block__mixer_token_mlp__prompt_kernel(
    A_x: jax.Array,
    A_wqkv: jax.Array,
    A_wo: jax.Array,
    B_x: jax.Array,
    B_w1: jax.Array,
    B_b1: jax.Array,
    B_w2: jax.Array,
    B_b2: jax.Array,
):
    del B_x
    hbm_spec = pl.BlockSpec(memory_space=pltpu.MemorySpace.HBM)
    vmem_spec = pl.BlockSpec(memory_space=pltpu.VMEM)
    scratch = [
        pltpu.VMEM((D, S), BF),
        pltpu.VMEM((D, 3 * D), BF),
        pltpu.VMEM((D, D), BF),
        pltpu.VMEM((S, F), BF),
        pltpu.VMEM((F, S), BF),
        pltpu.VMEM((3 * D, D), BF),
        pltpu.VMEM((HP, D), BF),
        pltpu.VMEM((D, HP), BF),
        pltpu.VMEM((2, D, RC), BF),
        pltpu.VMEM((H, S, DH), BF),
        pltpu.VMEM((HP, S), BF),
        pltpu.VMEM((HP, S), BF),
        pltpu.VMEM((S, TQ), F32),
        pltpu.VMEM((S, TQ), F32),
        pltpu.VMEM((1, TQ), F32),
        pltpu.VMEM((1, TQ), F32),
        pltpu.VMEM((HP, S), BF),
        pltpu.VMEM((D, S), F32),
        pltpu.VMEM((D, S), BF),
        pltpu.VMEM((D, F), BF),
        pltpu.VMEM((D, S), BF),
        pltpu.SemaphoreType.DMA((6 + S // RC,)),
        pltpu.SemaphoreType.DMA((S // SC,)),
    ]
    xT = jnp.swapaxes(A_x, 1, 2)
    outT = pl.pallas_call(
        _kernel,
        out_shape=jax.ShapeDtypeStruct((1, D, S), BF),
        in_specs=[hbm_spec, hbm_spec, hbm_spec, hbm_spec, vmem_spec, hbm_spec, vmem_spec],
        out_specs=hbm_spec,
        scratch_shapes=scratch,
        compiler_params=pltpu.CompilerParams(vmem_limit_bytes=110 * 1024 * 1024),
    )(xT, A_wqkv, A_wo, B_w1, B_b1, B_w2, B_b2)
    return jnp.swapaxes(outT, 1, 2)
```
